```python
import os as _os
_os.environ.setdefault("JAX_PLATFORMS", "cpu")
import jax
import jax.numpy as jnp

def _softmax(x, axis=-1):
    return jax.nn.softmax(x, axis=axis)
def _gelu(x):
    return jax.nn.gelu(x, approximate=True)
def _silu(x):
    return jax.nn.silu(x)
def _sigmoid(x):
    return jax.nn.sigmoid(x)
def _layernorm(x, axis=-1, eps=1e-5):
    m = jnp.mean(x, axis=axis, keepdims=True)
    v = jnp.var(x, axis=axis, keepdims=True)
    return (x - m) / jnp.sqrt(v + eps)
def _scatter_add(tgt, idx, src, axis=0):
    return tgt.at[idx].add(src)
def _segment_sum(src, seg, n):
    return jax.ops.segment_sum(src, seg, n)
class _Rng:
    def __init__(self, key):
        self._k = key
    def _next(self):
        self._k, sub = jax.random.split(self._k)
        return sub
    def normal(self, shape):
        return jax.random.normal(self._next(), shape, dtype=jnp.bfloat16)
    def randint(self, lo, hi, shape):
        return jax.random.randint(self._next(), shape, lo, hi, dtype=jnp.int32)
    def uniform(self, shape, lo=0.0, hi=1.0):
        return jax.random.uniform(self._next(), shape, jnp.bfloat16, lo, hi)
    def permutation(self, n):
        return jax.random.permutation(self._next(), n)


kernel_name = 'parallel_sum__sliding_local_dilated__geglu_ffn__prompt'

def setup_inputs():
    _rng = _Rng(jax.random.key(int.from_bytes(__import__("os").urandom(4), "little")))
    _w = (lambda a: (lambda t: t.astype(jnp.bfloat16) if jnp.issubdtype(t.dtype, jnp.floating) else t)(jnp.asarray(a)))
    def _A_setup():
        B, S, D = 1, 2048, 640
        return {
            "x": _w((lambda *s: _rng.normal(s) * 0.05)(B, S, D)),
            "wqkv": _w((lambda *s: _rng.normal(s) * 0.05)(D, 3 * D)),
            "wo": _w((lambda *s: _rng.normal(s) * 0.05)(D, D)),
        }
    _A_in = _A_setup()

    def _B_setup():
        B, S, D, F = 1, 2048, 640, 1728
        return {
            "x": _w((lambda *s: _rng.normal(s) * 0.05)(B, S, D)),
            "w_gate": _w((lambda *s: _rng.normal(s) * 0.05)(D, F)),
            "w_up": _w((lambda *s: _rng.normal(s) * 0.05)(D, F)),
            "w_down": _w((lambda *s: _rng.normal(s) * 0.05)(F, D)),
        }
    _B_in = _B_setup()

    return {
        "A_x": _A_in["x"],
        "A_wqkv": _A_in["wqkv"],
        "A_wo": _A_in["wo"],
        "B_x": _B_in["x"],
        "B_w_gate": _B_in["w_gate"],
        "B_w_up": _B_in["w_up"],
        "B_w_down": _B_in["w_down"],
    }

def reference(A_x, A_wqkv, A_wo, B_x, B_w_gate, B_w_up, B_w_down):
    def _A_ref(x, wqkv, wo):
        B, S, D = x.shape
        H = 32; Dh = D // H
        W, dil = 8, 2
        qkv = (lambda x, *d: x.transpose(*d))((x @ wqkv).reshape(B, S, 3, H, Dh), 2, 0, 3, 1, 4)
        q, k, v = qkv[0], qkv[1], qkv[2]
        scale = Dh ** -0.5
        pos = jnp.arange(S)
        off = jnp.arange(W) * dil
        idx = pos[:, None] - off[None, :]
        mask = idx >= 0
        idx_c = jnp.where(mask, idx, 0).reshape(-1)
        kg = k[:, :, idx_c, :].reshape(B, H, S, W, Dh)
        vg = v[:, :, idx_c, :].reshape(B, H, S, W, Dh)
        logits = jnp.einsum("bhsd,bhswd->bhsw", q, kg) * scale
        logits = jnp.where(mask[None, None, :, :], logits, -1e9)
        attn = _softmax(logits, axis=-1)
        o = jnp.einsum("bhsw,bhswd->bhsd", attn, vg)
        return (lambda x, *d: x.transpose(*d))(o, 0, 2, 1, 3).reshape(B, S, D) @ wo

    def _B_ref(x, w_gate, w_up, w_down):
        return (_gelu(x @ w_gate) * (x @ w_up)) @ w_down

    x = A_x
    xn = _layernorm(x, axis=-1)
    return x + _A_ref(xn, A_wqkv, A_wo) + _B_ref(xn, B_w_gate, B_w_up, B_w_down)
```

```python
import functools
import numpy as np
import jax
import jax.numpy as jnp
import jax.experimental.pallas as pl
import jax.experimental.pallas.tpu as pltpu

S, D, F, H, DH, WIN, DIL = 2048, 640, 1728, 32, 20, 8, 2
NT = D // 128
HALO = 16
FG = 12 * 128
FM = 13 * 128
FT = F - FM
bf16, f32 = jnp.bfloat16, jnp.float32
_LATER = object()
_NN = (((1,), (0,)), ((), ()))
_NT = (((1,), (1,)), ((), ()))

_ALG = (
    (((0, 'a', 1),), ((0, 0, 1), (0, 2, 1), (1, 0, 1)), ((0, 'c', 1),)),
    (((0, 'c', 1),), ((0, 0, 1), (0, 1, 1), (2, 0, 1)), ((0, 'a', 1),)),
    (((1, 'b', 1),), ((0, 1, 1), (1, 1, 1), (1, 2, 1)), ((1, 'c', 1),)),
    (((1, 'c', 1),), ((1, 0, 1), (1, 1, 1), (2, 1, 1)), ((1, 'b', -1),)),
    (((1, 'b', 1), (0, 'b', -1)), ((0, 1, 1),), ((0, 'a', 1), (1, 'a', -1))),
    (((1, 'a', 1), (0, 'a', -1)), ((1, 0, 1),), ((0, 'b', 1), (1, 'b', -1))),
    (((1, 'b', 1), (0, 'a', -1)), ((1, 0, 1), (0, 1, -1)), ((0, 'a', 1), (1, 'b', 1))),
    (((2, 'b', 1),), ((0, 2, 1), (2, 1, 1), (2, 2, 1)), ((2, 'a', 1),)),
    (((2, 'a', 1),), ((1, 2, 1), (2, 0, 1), (2, 2, 1)), ((2, 'b', 1),)),
    (((2, 'b', 1), (0, 'b', -1)), ((0, 2, 1),), ((0, 'c', 1), (2, 'c', -1))),
    (((2, 'c', 1), (0, 'c', -1)), ((2, 0, 1),), ((0, 'b', -1), (2, 'b', 1))),
    (((2, 'b', 1), (0, 'c', -1)), ((2, 0, 1), (0, 2, -1)), ((0, 'c', 1), (2, 'b', -1))),
    (((2, 'a', 1), (1, 'a', -1)), ((1, 2, 1),), ((1, 'c', 1), (2, 'c', -1))),
    (((2, 'c', 1), (1, 'c', -1)), ((2, 1, 1),), ((1, 'a', 1), (2, 'a', -1))),
    (((2, 'a', 1), (1, 'c', 1)), ((2, 1, 1), (1, 2, -1)), ((1, 'c', 1), (2, 'a', -1))),
)


def _signed_sum(terms):
    first = [s for _, s in terms].index(1)
    acc = terms[first][0]
    for v, s in terms[:first] + terms[first + 1:]:
        acc = acc + v if s > 0 else acc - v
    return acc


def _lhs_ops(top, bot):
    pt = [dict(a=b, b=t, c=t - b) for t, b in zip(top, bot)]
    return (_signed_sum([(pt[k][p], s) for k, p, s in l]) for l, _, _ in _ALG[:15 if len(top) == 3 else 7])


def _rhs_ops(blk):
    n_blk = len(blk)
    wide = [[b.astype(f32) for b in row] for row in blk]
    for _, r, _ in _ALG[:15 if n_blk == 3 else 7]:
        r = [(k, n, s) for k, n, s in r if k < n_blk and n < n_blk]
        yield blk[r[0][0]][r[0][1]] if len(r) == 1 else _signed_sum([(wide[k][n], s) for k, n, s in r]).astype(bf16)


def _signed_add(a, b):
    if a is None:
        return b
    if a[1] == b[1]:
        return a[0] + b[0], a[1]
    return (a[0] - b[0], 1) if a[1] > 0 else (b[0] - a[0], 1)


def _scatter(acc, m, val, tiles):
    for n, p, s in _ALG[m][2]:
        acc[(tiles[n], p)] = _signed_add(acc.get((tiles[n], p)), (val, s))


def _gather(acc, tile):
    out = [_signed_add(acc[(tile, p)], acc[(tile, 'c')]) for p in 'ab']
    assert all(s > 0 for _, s in out)
    return [v for v, _ in out]


class _Tiled:
    def __init__(self, ref):
        self.ref = ref

    def _idx(self, idx):
        r = idx[0]
        r0, r1 = (r.start, r.start + r.size) if isinstance(r, pl.Slice) else r.indices(2 * self.ref.shape[0])[:2]
        return slice(r0 // 2, r1 // 2), idx[1]

    def __getitem__(self, idx):
        return pltpu.bitcast(self.ref[self._idx(idx)], bf16)

    def __setitem__(self, idx, val):
        self.ref[self._idx(idx)] = val if val.dtype == jnp.uint32 else pltpu.bitcast(val, jnp.uint32)


def _gelu(g):
    c0 = float(np.sqrt(2.0 / np.pi))
    t = jnp.tanh(g * (c0 + (c0 * 0.044715) * (g * g)))
    hg = 0.5 * g
    return hg + hg * t


def _gelu_mul(g, u):
    return _gelu(g) * u


def _dot(a, b, dims=_NN):
    return jax.lax.dot_general(a, b, dims, preferred_element_type=f32)


def _t(n):
    return slice(n * 128, (n + 1) * 128)


def _share(tasks, weights):
    cum = np.cumsum((0,) + tuple(weights)) * len(tasks) // sum(weights)
    return [tasks[a:b] for a, b in zip(cum[:-1], cum[1:])]


K1 = [256] * 7 + [128] * 8
O1 = [int(v) for v in np.cumsum([0] + K1)]


def make(NF=256, TM=448, AR=8, LR=16, flags=None, gord=(0, 1, 3, 4, 5, 6, 2), qk_sp=(2, 1, 1, 1, 1, 0), pv_sp=(1, 2, 1),
         cb_sp=(0, 1, 1), h_late=0, ln_sp=(2, 1), sp2=0.85, peel=True, dl={}, SB=7, sp3=0.1, q0_sp=(2, 1), n0_sp=(1, 1, 1), PR=32, cut2=(8, 10), trail=16, span=0.92, span0=0.8, ord1=tuple(range(22)), ord2=tuple(range(15))):
    dl = {**dict(n=12, h=16, x=12, p=8, w=0, m=0), **dl}
    nt = (S - NF) // TM
    assert NF + nt * TM == S and NF <= TM
    HM = TM // 2
    scale = DH ** -0.5
    c_exp = scale * float(np.log2(np.e))
    P = functools.partial

    def kernel(x_hbm, wqkv_hbm, wo_hbm, wg_hbm, wu_hbm, wd_hbm, o_hbm,
               x_s, o_s, wqkv, wo_raw, wo_f, wgu, wt, wd, wp, wop, r_dn, b1n, b1t, b2, b2x,
               xn0, a1, a2a, a2c, a2x, a2xo, a2r, h0, h0o, h_s, ao, l_s, p_s, y_s, xn_s, pr, q_s, k_s, v_s,
               sem_i, sem_o):
        wp = [_Tiled(r) for r in wp]
        wop, r_dn, b1n, b1t, b2, b2x, xn0, a1, a2a, a2c, a2x, a2xo, a2r, h0, h0o = map(
            _Tiled, (wop, r_dn, b1n, b1t, b2, b2x, xn0, a1, a2a, a2c, a2x, a2xo, a2r, h0, h0o))
        copies = []

        def fetch(src, dst):
            copies.append(pltpu.make_async_copy(src, dst, sem_i.at[len(copies)]))
            return copies[-1]

        def fetch_rows(src, dst, r, n):
            return fetch(src.at[pl.ds(r, n)], dst.at[pl.ds(r, n)])

        def fetch_gu(g):
            return [fetch(src.at[pl.ds(g * 384, 384)], wgu[g].at[pl.ds(o, 384)])
                    for src, o in ((wg_hbm, 0), (wu_hbm, 384))]

        def fetch_qkv(p):
            return fetch(wqkv_hbm.at[:, pl.ds(p * D, D)], wqkv[p].at[pl.ds(0, D)])
        cp_x0 = fetch_rows(x_hbm, x_s, 0, NF)
        cp_gu, cp_qkv = [], []
        for g in range(3):
            cp_gu.append(fetch_gu(g))
            cp_qkv.append(fetch_qkv(g))
        cp_t = [fetch(wg_hbm.at[pl.ds(FM, FT)], wt.at[pl.ds(0, FT)]),
                fetch(wu_hbm.at[pl.ds(FM, FT)], wt.at[pl.ds(FT, FT)]),
                fetch(wg_hbm.at[pl.ds(FG, 128)], wt.at[pl.ds(128, 128)]),
                fetch(wu_hbm.at[pl.ds(FG, 128)], wt.at[pl.ds(256, 128)])]
        cp_gu.append(fetch_gu(3))
        cp_d = [fetch(wd_hbm.at[pl.ds(0, 768)], wd[0].at[pl.ds(0, 768)])]
        cp_x1 = fetch_rows(x_hbm, x_s, NF, TM)
        cp_d.append(fetch(wd_hbm.at[pl.ds(768, F - 768)], wd[1].at[pl.ds(0, F - 768)]))
        cp_wo = fetch(wo_hbm, wo_raw.at[pl.ds(0, D)])
        cp_x2 = fetch_rows(x_hbm, x_s, NF + TM, S - NF - TM)

        def cp_o(r, n, s):
            return pltpu.make_async_copy(o_s.at[pl.ds(r, n)], o_hbm.at[pl.ds(r, n)], sem_o.at[s])

        zero = []
        pending = []
        clock = [0.0]
        made = set()

        def missing(stage, *spans):
            return any((stage, r) not in made for r0, r1 in spans for r in range(max(r0, 0), r1, 8))

        def fence(val, *refs):
            for ref in refs:
                if val is None:
                    return
                ref = ref.ref if isinstance(ref, _Tiled) else ref
                n = 16 if ref.dtype == bf16 else 8
                v = pltpu.bitcast(val[0:16 if val.dtype == bf16 else 8], ref.dtype)
                rows = pl.ds(pl.multiple_of(ref.shape[-2] - n + zero[0], n), n)
                ref[(0,) * (len(ref.shape) - 2) + (rows, slice(0, 128))] = v

        def done(kind, *refs):
            if not dl.get(kind):
                return None
            val = jnp.zeros((8, 128), f32)
            for ref in refs:
                fence(val, ref)
                ref = ref.ref if isinstance(ref, _Tiled) else ref
                val = ref[(0,) * (len(ref.shape) - 2) + (slice(ref.shape[-2] - 8, None), slice(0, 128))]
            return dl[kind], val

        def phase(dots, *task_lists, span=span):
            total = sum(d[1] for d in dots)
            todo = sorted((clock[0] + s / len(ts) * span * total, n, s)
                          for n, ts in enumerate(task_lists) for s in range(len(ts)))
            out = []
            dots = list(dots)
            while dots:
                for due in [d for d in pending if d[0] <= clock[0]]:
                    fence(due[2], dots[0][2])
                pending[:] = [d for d in pending if d[0] > clock[0]]
                cost, first = 0, len(out)
                while dots and cost < 3:
                    cost += dots[0][1]
                    out.append(dots.pop(0)[0]())
                m = out[first]
                for at, n, s in [t for t in todo if t[0] < clock[0] + cost]:
                    r = min(int(max(at - clock[0], 0) / cost * m.shape[0]) // 16 * 16, m.shape[0] - 16)
                    res = task_lists[n][s](m[r:r + 16, 0:128])
                    if res is not _LATER:
                        todo.remove((at, n, s))
                        if res is not None:
                            pending.append((max(at, clock[0]) + res[0], n, res[1]))
                clock[0] += cost
            for _, n, s in todo:
                res = task_lists[n][s](None)
                assert res is not _LATER
            return out

        def perm_qkv(p, r, tok):
            lane = jax.lax.broadcasted_iota(jnp.int32, (PR // 2, 128), 1)
            m_of = 4 * (lane % 32) + lane // 32
            fence(tok, wqkv[p])
            src = [pltpu.bitcast(wqkv[p][r:r + PR, _t(i)], jnp.uint32) for i in range(NT)]
            for j in range(NT):
                t = src[0]
                for i in range(1, NT):
                    t = jnp.where(lane % NT == (j - 128 * i) % NT, src[i], t)
                t = jnp.take_along_axis(t, (NT * m_of + j) % 128, axis=1, mode='promise_in_bounds')
                wp[p][r:r + PR, _t(j)] = t
            return done('m', wp[p])

        def tail_t(j, tok):
            wp[3][0:D, _t(j)] = wt[_t(j), :].astype(f32).T.astype(bf16)

        def prep1(g, s, r, tok):
            if g < 3:
                fence(tok, wp[g], wp[g + 1])

                def get(k, n):
                    return wp[(6 * g + n) // NT][pl.ds(r + k * 128, 16), _t((6 * g + n) % NT)]

                def put(ko, n, v):
                    b1n[ko + r:ko + r + 16, _t(3 * g + n)] = v
            else:
                fence(tok, wgu[g - 3])

                def get(k, n):
                    return wgu[g - 3][pl.ds(r + n % 2 * 384 + n // 2 * 128, 16), _t(k)]

                def put(ko, n, v):
                    b1t[pl.ds((g - 3) * 384 + n * 128 + r, 16), ko:ko + 128] = v
            todo = ([((0, 1, 2), (s, 2 + s, 4 + s), 0, s)] if s < 2 else
                    [((3, 4), ns, 128, j) for j, ns in enumerate(((0, 2), (1, 3), (4, 5)))])
            for ks, ns, o, j in todo:
                for m, v in enumerate(_rhs_ops([[get(k, n) for n in ns] for k in ks])):
                    put(O1[m] + o, j, v)
            return done('w', b1n if g < 3 else b1t)

        def widen_wo(_, r, tok):
            fence(tok, wo_raw)
            v = wo_raw[r:r + 64, :].astype(f32)
            for j in range(NT):
                wo_f[j, r:r + 64, :] = v[:, _t(j)]

        def perm_wo(j, tok):
            fence(tok, wo_f)
            for r4 in range(4):
                for i in range(NT):
                    wop[j * 128 + r4 * 32:j * 128 + (r4 + 1) * 32, _t(i)] = (
                        wo_f[i, pl.ds(NT * r4 + j, H, stride=DH), :].astype(bf16))

        def prep2(gg, s, r, tok):
            fence(tok, (wd[0], wd[1], wop)[gg])

            def get(k, n):
                src, o = (wd[0], k) if k < 6 else (wd[1], k - 6) if k < 13 else (wop, k - 13)
                return src[pl.ds(r + o * 128, 16), _t(n)]
            todo = ([((3 * s, 3 * s + 1, 3 * s + 2), (0, 1, 2), b2, 2 * gg + s, 0)] if s < 2 else
                    [((2, 5), (3, 4), b2x, gg, 0), ((0, 1), (3, 4), b2, 2 * gg, 15), ((3, 4), (3, 4), b2, 2 * gg + 1, 15)])
            for ks, ns, dst, j, c in todo:
                for m, v in enumerate(_rhs_ops([[get(6 * gg + k, n) for n in ns] for k in ks])):
                    dst[pl.ds(j * 128 + r, 16), _t(c + m)] = v
            return done('w', b2)

        def ln(r0):
            x = x_s[pl.ds(r0, LR), :].astype(f32)
            xc = x - jnp.sum(x, axis=-1, keepdims=True) * (1.0 / D)
            var = jnp.sum(xc * xc, axis=-1, keepdims=True) * (1.0 / D)
            return xc * jax.lax.rsqrt(var + 1e-5)

        def normalize(base, r, tok):
            fence(tok, x_s)
            xn_s[r:r + LR, :] = v = ln(pl.multiple_of(base + r, 16))
            made.update(('xn', r0) for r0 in range(r, r + LR, 8))
            return done('n', xn_s)

        def x_ops(ks, r, tok):
            if missing('xn', (r, r + 16), (HM + r, HM + r + 16)):
                return _LATER
            fence(tok, xn_s)
            o = 128 if len(ks) == 2 else 0
            for m, a in enumerate(_lhs_ops(*[[xn_s[r0:r0 + 16, _t(k)] for k in ks] for r0 in (r, HM + r)])):
                a1[r:r + 16, O1[m] + o:O1[m] + o + 128] = a.astype(bf16)
            return done('x', a1)
        x_tasks = [P(x_ops, ks, r) for r in range(0, HM, 16) for ks in ((0, 1, 2), (3, 4))]

        def gelu_tail(val):
            lane = jax.lax.broadcasted_iota(jnp.int32, val.shape, 1)
            return jnp.where(lane < FT, _gelu_mul(val, pltpu.roll(val, FT, 1)), 0.0)

        def quarters(n):
            lane = jax.lax.broadcasted_iota(jnp.int32, (n, 128), 1)
            return lane, lane % 64 < 32, lane < 64

        def attn_qk(r, c, tok):
            if missing(0, (r, r + 8)) or missing(1, (r - HALO, r + 8)):
                return _LATER
            fence(tok, q_s, k_s)
            made.add((('l', c), r))
            _, even, low = quarters(8)
            q = [q_s[j, r:r + 8, :] for j in range(NT)]

            def part(w):
                return functools.reduce(
                    jnp.add, (q[j] * k_s[j, pl.ds(HALO + r - DIL * w, 8), :] for j in range(NT)))

            def fold(sel, a, b, shift):
                return jnp.where(sel, a, b) + pltpu.roll(jnp.where(sel, b, a), shift, 1)
            u = [fold(even, part(w), part(w + 1), 32) for w in (4 * c, 4 * c + 2)]
            l_s[r:r + 8, _t(c)] = fold(low, u[0], u[1], 64)
            return done('q', l_s)

        def softmax(rs, first, tok):
            if any(missing(('l', c), (r, r + 16)) for r in rs for c in range(2)):
                return _LATER
            fence(tok, l_s)
            made.update(('p', r + o) for r in rs for o in (0, 8))
            lg = [[l_s[r:r + 16, _t(c)] for r in rs] for c in range(2)]
            if first:
                row = jax.lax.broadcasted_iota(jnp.int32, (16, 128), 0)
                for c in range(2):
                    lg[c][0] = jnp.where(row >= DIL * (4 * c + quarters(16)[0] // 32), lg[c][0], -1e9 / scale)
            lg = [jnp.concatenate(v, axis=0) for v in lg]

            def all_reduce(op, v):
                v = op(v[0], v[1])
                v = op(v, pltpu.roll(v, 64, 1))
                return op(v, pltpu.roll(v, 32, 1))
            mx = all_reduce(jnp.maximum, lg)
            e = [jnp.exp2((v - mx) * c_exp) for v in lg]
            inv = 1.0 / all_reduce(jnp.add, e)
            for c in range(2):
                for n, r in enumerate(rs):
                    p_s[r:r + 16, _t(c)] = e[c][16 * n:16 * n + 16] * inv[16 * n:16 * n + 16]
            return done('s', p_s)

        def logits(rows, first):
            out = []
            for n, r in enumerate(rows + [None]):
                if r is not None:
                    out += [P(attn_qk, r + o, c) for o in (0, 8) for c in range(2)]
                if n > 0 and (n % SB == 0 or r is None):
                    n0 = (n - 1) // SB * SB
                    out.append(P(softmax, rows[n0:n], first and n0 == 0))
            return out

        def attn_pv(r, tok):
            if missing('p', (r, r + 8)) or missing(2, (r - HALO, r + 8)):
                return _LATER
            fence(tok, p_s, v_s)
            made.add(('o', r))
            _, even, low = quarters(8)

            def spread(sel, z, shift):
                y = pltpu.roll(z, shift, 1)
                return jnp.where(sel, z, y), jnp.where(sel, y, z)
            p = [b for c in range(2) for a in spread(low, p_s[r:r + 8, _t(c)], 64) for b in spread(even, a, 32)]
            for j in range(NT):
                ao[r:r + 8, _t(1 + j)] = functools.reduce(
                    jnp.add, (p[w] * v_s[j, pl.ds(HALO + r - DIL * w, 8), :] for w in range(WIN)))
            return done('p', ao)

        def attn_ops(s, r, tok):
            if missing('o', (r, r + 16), (HM + r, HM + r + 16)):
                return _LATER
            fence(tok, ao)
            t, b = [[ao[pl.ds(r + o, 16), _t(j)] for j in ((0, 1, 2), (3, 4, 5), (2, 5))[s]] for o in (0, HM)]
            for m, a in enumerate(_lhs_ops(t, b)):
                (a2c if s < 2 else a2xo)[r:r + 16, _t(2 * m + s if s < 2 else m)] = a.astype(bf16)
            if s == 2:
                for o in (r, r + HM):
                    a2r[o:o + 16, :] = ao[o:o + 16, _t(6)].astype(bf16)
            return done('c', a2c if s < 2 else a2xo)

        def mm1(g):
            def one(ks, n0, n1, c):
                if g < 3:
                    p = _dot(a1[0:HM, ks], b1n[ks, g * 384 + n0:g * 384 + n1])
                else:
                    p = _dot(a1[0:HM, ks], b1t[(g - 3) * 384 + n0:(g - 3) * 384 + n1, ks], _NT)
                pr[gord.index(g) % 2][0:HM, c * 128:c * 128 + n1 - n0] = p
                return p
            return [(P(one, slice(O1[m], O1[m + 1]), 0, 256, 2 * m) if m < 15 else
                     P(one, slice(O1[m - 15] + 128, O1[m - 15] + 256), 256, 384, 15 + m),
                     K1[m] // 64 if m < 15 else 1, b1n if g < 3 else b1t) for m in ord1]

        def epi1(g, r, tok):
            fence(tok, pr[gord.index(g) % 2])
            made.update(((g, r), (g, HM + r)))
            acc, res = {}, {}
            for m in range(7):
                _scatter(acc, m, pr[gord.index(g) % 2][r:r + 8, _t(30 + m)], (4, 5))
            for s in range(2):
                for m in range(15):
                    _scatter(acc, m, pr[gord.index(g) % 2][r:r + 8, _t(2 * m + s)], (s, 2 + s, 4 + s))
                for c in range(s, 6, 2):
                    n = 6 * g + c
                    for r0, val in zip((r, HM + r), _gather(acc, c)):
                        if n < NT:
                            q_s[n, r0:r0 + 8, :] = val
                        elif n < 15:
                            (k_s, v_s)[n // NT - 1][n % NT, HALO + r0:HALO + r0 + 8, :] = val
                        elif n == 15:
                            ao[r0:r0 + 8, _t(6)] = gelu_tail(val)
                        elif s == 0:
                            res[(c, r0)] = _gelu(val)
                        else:
                            val = res[(c - 1, r0)] * val
                            (ao if g == 2 else h_s)[r0:r0 + 8, _t(0 if g == 2 else n // 2 - 9)] = val
            return done('e', (q_s, k_s, ao, h_s)[min(g, 3)])

        def h_ops(g, r, tok):
            fence(tok, h_s)
            t, b = [[h_s[pl.ds(r + o, 16), _t(3 * g + k)] for k in range(3)] for o in (0, HM)]
            for m, a in enumerate(_lhs_ops(t, b)):
                a2a[r:r + 16, _t(4 * m + g)] = a.astype(bf16)
            if g % 2 == 1:
                t0, b0 = [h_s[pl.ds(r + o, 16), _t(3 * g - 1)] for o in (0, HM)]
                for m, a in enumerate(_lhs_ops([t0, t[2]], [b0, b[2]])):
                    a2x[r:r + 16, _t(2 * m + g // 2)] = a.astype(bf16)
            return done('h', *[a2a] + [a2x] * (g % 2))

        def epis(g):
            out = []
            for r in range(0, HM + trail, 16):
                if r < HM:
                    out += [P(epi1, g, r), P(epi1, g, r + 8)]
                if g >= 3 and r >= trail:
                    out.append(P(h_ops, g - 3, r - trail))
            return out

        def epi2(src, n_prod, tiles, r, tok):
            fence(tok, src)
            acc = {}
            for m in range(n_prod):
                _scatter(acc, m, src[r:r + 8, _t(m)], tiles)
            for n in tiles:
                for o, val in zip((r, HM + r), _gather(acc, n)):
                    y_s[n > 2][o:o + 8, _t(n)] = val

        def tile(i, carry):
            base = pl.multiple_of(NF + i * TM, 32)
            nxt = NF + jnp.minimum(i + 1, nt - 1) * TM
            k_s[:, 0:HALO, :] = k_s[:, TM:TM + HALO, :]
            v_s[:, 0:HALO, :] = v_s[:, TM:TM + HALO, :]
            rows = sorted(range(0, TM, 16), key=lambda r: r % HM or HM // 2)
            qk = _share(logits(rows, False), qk_sp)
            rows = sorted(range(0, HM, 16), key=lambda r: r or HM // 2)
            pv = _share([P(attn_pv, o + r) for r in rows for o in (0, 8, HM, HM + 8)], pv_sp)
            cb = _share([P(attn_ops, s, r) for r in rows for s in range(3)], cb_sp)
            lns = _share([P(normalize, nxt, r) for r in range(0, TM, LR)], ln_sp)
            pending.clear()
            made.clear()
            phase(mm1(0), lns[0])
            phase(mm1(1), epis(0), lns[1])
            idle = [lambda tok: None] * 2
            for n in range(2, 7):
                phase(mm1(gord[n]), epis(gord[n - 1]), idle * (3 * (n == 2)) + qk[n - 2])

            def mm2(m, n, acc, dst, lhs, rhs):
                p = _dot(jnp.concatenate([a[0:HM, (w * m + w0) * 128:(w * m + w1) * 128] for a, w, w0, w1 in lhs], axis=1),
                         jnp.concatenate([b[k0:k1, _t(c + m)] for b, k0, k1, c in rhs], axis=0))
                p = p if acc is None else acc[n] + p
                if dst is not None:
                    dst[0:HM, _t(m)] = p
                return p

            def mm2s(ms, *a):
                return [(P(mm2, m, n, *a), sum(w1 - w0 for _, _, w0, w1 in a[2]), b2) for n, m in enumerate(ms)]
            d = mm2s(ord2, None, None, [(a2a, 4, 0, 4)], [(b2, 0, 512, 0)])
            p = phase(d[:cut2[0]], epis(2), qk[5] + idle + pv[0], span=1)
            d = d[cut2[0]:] + mm2s(range(7), None, None, [(a2a, 4, 0, 4)], [(b2, 0, 512, 15)])
            p += phase(d[:cut2[1]], pv[1], cb[0] + cb[1], span=1)
            p += phase(d[cut2[1]:] + mm2s(range(7), None, None, [(a2x, 2, 0, 2)], [(b2x, 0, 256, 0)]),
                       pv[2] + idle * 2, cb[2], span=sp2)
            phase(mm2s(ord2, p, pr[0], [(a2c, 2, 0, 2)], [(b2, 512, 768, 0)]), x_tasks)
            phase(mm2s(range(7), [p[15 + m] + p[22 + m] for m in range(7)], pr[1],
                       [(a2c, 2, 0, 2), (a2xo, 1, 0, 1)], [(b2, 512, 768, 15), (b2x, 256, 384, 0)]),
                  [P(epi2, pr[0], 15, (0, 1, 2), r) for r in range(0, HM, 8)])

            def last(c0, c1):
                e = _dot(a2r[:, :], r_dn[:, c0:c1])
                o_s[pl.ds(base, TM), c0:c1] = (y_s[c0 > 0][:, c0:c1] + x_s[pl.ds(base, TM), c0:c1].astype(f32)
                                               + e).astype(bf16)
                return e
            pending.clear()
            phase([(P(last, 0, 384), 6, None)], [P(epi2, pr[1], 7, (3, 4), r) for r in range(0, HM, 8)], span=sp3)
            last(384, 640)
            cp_o(base, TM, i + 1).start()
            return carry

        for c in copies:
            c.start()
        cp_x0.wait()
        bits = jax.lax.population_count(jax.lax.bitcast_convert_type(x_s[0:16, 0:128].astype(f32), jnp.int32))
        zero.append(bits[0, 0] >> 6)
        for r in range(0, NF, LR):
            xn0[r:r + LR, :] = ln(r).astype(bf16)
        o0 = TM - NF

        def strips(f, a, n):
            return [P(f, a, r) for r in range(0, D, n)]

        def prep(f, a):
            return [P(f, a, s, r) for r in range(0, 128, 16) for s in range(3)]

        if not peel:
            jax.lax.fori_loop(0, nt, tile, None)
            return

        def wait(*cs):
            pending.clear()
            for c in cs:
                c.wait()

        def gu0(g):
            def one(k):
                w = jnp.concatenate([wgu[g][_t(k), :], wgu[g][_t(3 + k), :]], axis=0)
                res = _dot(xn0[:, :], w, _NT)
                h0[:, _t(3 * g + k)] = _gelu_mul(res[:, :128], res[:, 128:]).astype(bf16)
                return res
            return [(P(one, k), 10, wgu[g]) for k in range(3)]

        def qkv0(p):
            dst, o = ((q_s, o0), (k_s, o0 + HALO), (v_s, o0 + HALO))[p]

            def one(j):
                dst[j, o:o + NF, :] = res = _dot(xn0[:, :], wp[p][0:D, _t(j)])
                if p > 0:
                    dst[j, o0:o, :] = jnp.broadcast_to(res[0:1], (HALO, 128))
                return res
            return [(P(one, j), 5, wp[p]) for j in range(NT)]

        def tail0():
            res = _dot(xn0[:, :], wt[...], _NT)
            h0[:, FG:FM] = _gelu_mul(res[:, _t(1)], res[:, _t(2)]).astype(bf16)
            a2r[0:NF, :] = gelu_tail(res[:, _t(0)]).astype(bf16)
            return res

        def down0(acc, a, k0, k1, b):
            return [(lambda j=j: acc(j) + _dot(a[0:NF, k0:k1], b[0:k1 - k0, _t(j)]), (k1 - k0) // 128, b)
                    for j in range(NT)]

        def attn0(r, tok):
            h0o[r:r + 16, :] = ao[o0 + r:o0 + r + 16, 128:128 + D].astype(bf16)
        qk = _share(logits(list(range(o0, TM, 16)), True), q0_sp)
        nrm = _share([P(normalize, NF, r) for r in range(0, TM, LR)], n0_sp)
        made.update((g, r) for g in range(3) for r in range(0, TM, 8))
        wait(*cp_gu[0])
        phase(gu0(0))
        wait(cp_qkv[0], *cp_gu[1])
        phase(gu0(1), strips(perm_qkv, 0, PR), span=span0)
        wait(cp_qkv[1])
        phase(qkv0(0), strips(perm_qkv, 1, PR), prep(prep1, 3), span=span0)
        wait(cp_qkv[2], *cp_gu[2])
        phase(gu0(2), prep(prep1, 0), span=1)
        phase(qkv0(1), strips(perm_qkv, 2, PR), prep(prep1, 4), span=span0)
        wait(*cp_t, *cp_gu[3])
        phase(qkv0(2), [P(tail_t, j) for j in range(3)] + prep(prep1, 5), qk[0], span=1)
        phase(gu0(3) + [(tail0, 15, wgu[3])], qk[1], prep(prep1, 1) + prep(prep1, 2), span=span0)
        wait(*cp_d, cp_x1, cp_wo, cp_x2)
        r_dn[0:FT, :] = wd[1][FM - 768:F - 768, :]
        r_dn[FT:, :] = jnp.zeros((128 - FT, D), bf16)
        y = phase(down0(lambda j: x_s[0:NF, _t(j)].astype(f32), h0, 768, FM, wd[1]),
                  strips(widen_wo, 0, 64) + [P(perm_wo, j) for j in range(NT)],
                  [P(attn_pv, r) for r in range(o0, TM, 8)], nrm[0], span=1)
        y = phase(down0(y.__getitem__, h0, 0, 768, wd[0]), [P(attn0, r) for r in range(0, NF, 16)],
                  prep(prep2, 1) + prep(prep2, 2), nrm[1], span=1)
        y = phase(down0(y.__getitem__, h0o, 0, D, wop) + [(lambda: _dot(a2r[0:NF, :], r_dn[:, :]), 5, wop)],
                  nrm[2] + x_tasks, prep(prep1, 6) + prep(prep2, 0), span=span0)
        for j in range(NT):
            o_s[0:NF, _t(j)] = (y[j] + y[NT][:, _t(j)]).astype(bf16)
        cp_o(0, NF, 0).start()
        jax.lax.fori_loop(0, nt, tile if peel == 1 else lambda i, c: fence(y[0], b1n, b1t, b2, a1, b2x), None)
        cp_o(0, NF, 0).wait()
        for i in range(nt):
            cp_o(NF + i * TM, TM, i + 1).wait()

    def fn(A_x, A_wqkv, A_wo, B_x, B_w_gate, B_w_up, B_w_down):
        hbm = pl.BlockSpec(memory_space=pl.ANY)
        V = pltpu.VMEM

        def T(rows, panels):
            return V((rows // 2, panels * 128), jnp.uint32)
        out = pl.pallas_call(
            kernel,
            in_specs=[hbm] * 6,
            out_specs=hbm,
            out_shape=jax.ShapeDtypeStruct((S, D), A_x.dtype),
            scratch_shapes=[
                V((S + 16, D), bf16), V((S, D), bf16), [V((D + 16, D), bf16)] * 3, V((D + 16, D), bf16),
                V((NT, D + 8, 128), f32), [V((768 + 16, D), bf16)] * 4, V((384, D), bf16),
                [V((F - 768 + 16, D), bf16)] * 2, [T(D + 16, NT)] * 4, T(D + 16, NT), T(128, NT),
                T(O1[15] + 16, 9), T(FG + 16, 22), T(768 + 16, 22), T(384, 7),
                T(NF, NT), T(HM + 16, 22), T(HM + 16, 60), T(HM + 16, 30),
                T(HM + 16, 14), T(HM + 16, 7), T(TM, 1),
                T(NF, 13), T(NF, NT), V((TM + 8, 12 * 128), f32), V((TM + 8, 7 * 128), f32),
                V((TM + 8, 256), f32), V((TM + 8, 256), f32), [V((TM, D), f32)] * 2, V((TM + 8, D), f32), [V((HM + 8, 37 * 128), f32)] * 2,
                V((NT, TM + 8, 128), f32), V((NT, HALO + TM + 8, 128), f32), V((NT, HALO + TM + 8, 128), f32),
                pltpu.SemaphoreType.DMA((21,)), pltpu.SemaphoreType.DMA((nt + 1,)),
            ],
            compiler_params=pltpu.CompilerParams(vmem_limit_bytes=110 * 1024 * 1024, flags=flags,
                                                 disable_bounds_checks=True),
        )(A_x.reshape(S, D), A_wqkv, A_wo, B_w_gate.T, B_w_up.T, B_w_down)
        return out.reshape(A_x.shape)
    return fn


_kernel_fn = make(NF=384, TM=416)


@jax.jit
def pallas_parallel_sum__sliding_local_dilated__geglu_ffn__prompt_kernel(
    A_x: jax.Array,
    A_wqkv: jax.Array,
    A_wo: jax.Array,
    B_x: jax.Array,
    B_w_gate: jax.Array,
    B_w_up: jax.Array,
    B_w_down: jax.Array,
):
    return _kernel_fn(A_x, A_wqkv, A_wo, B_x, B_w_gate, B_w_up, B_w_down)
```

```python
import functools
import numpy as np
import jax
import jax.numpy as jnp
import jax.experimental.pallas as pl
import jax.experimental.pallas.tpu as pltpu

S, D, F, H, DH, WIN, DIL = 2048, 640, 1728, 32, 20, 8, 2
NT = D // 128
HALO = 16
FG = 12 * 128
FM = 13 * 128
FT = F - FM
bf16, f32 = jnp.bfloat16, jnp.float32
_LATER = object()
_NN = (((1,), (0,)), ((), ()))
_NT = (((1,), (1,)), ((), ()))

_ALG = (
    (((0, 'a', 1),), ((0, 0, 1), (0, 2, 1), (1, 0, 1)), ((0, 'c', 1),)),
    (((0, 'c', 1),), ((0, 0, 1), (0, 1, 1), (2, 0, 1)), ((0, 'a', 1),)),
    (((1, 'b', 1),), ((0, 1, 1), (1, 1, 1), (1, 2, 1)), ((1, 'c', 1),)),
    (((1, 'c', 1),), ((1, 0, 1), (1, 1, 1), (2, 1, 1)), ((1, 'b', -1),)),
    (((1, 'b', 1), (0, 'b', -1)), ((0, 1, 1),), ((0, 'a', 1), (1, 'a', -1))),
    (((1, 'a', 1), (0, 'a', -1)), ((1, 0, 1),), ((0, 'b', 1), (1, 'b', -1))),
    (((1, 'b', 1), (0, 'a', -1)), ((1, 0, 1), (0, 1, -1)), ((0, 'a', 1), (1, 'b', 1))),
    (((2, 'b', 1),), ((0, 2, 1), (2, 1, 1), (2, 2, 1)), ((2, 'a', 1),)),
    (((2, 'a', 1),), ((1, 2, 1), (2, 0, 1), (2, 2, 1)), ((2, 'b', 1),)),
    (((2, 'b', 1), (0, 'b', -1)), ((0, 2, 1),), ((0, 'c', 1), (2, 'c', -1))),
    (((2, 'c', 1), (0, 'c', -1)), ((2, 0, 1),), ((0, 'b', -1), (2, 'b', 1))),
    (((2, 'b', 1), (0, 'c', -1)), ((2, 0, 1), (0, 2, -1)), ((0, 'c', 1), (2, 'b', -1))),
    (((2, 'a', 1), (1, 'a', -1)), ((1, 2, 1),), ((1, 'c', 1), (2, 'c', -1))),
    (((2, 'c', 1), (1, 'c', -1)), ((2, 1, 1),), ((1, 'a', 1), (2, 'a', -1))),
    (((2, 'a', 1), (1, 'c', 1)), ((2, 1, 1), (1, 2, -1)), ((1, 'c', 1), (2, 'a', -1))),
)


def _signed_sum(terms):
    first = [s for _, s in terms].index(1)
    acc = terms[first][0]
    for v, s in terms[:first] + terms[first + 1:]:
        acc = acc + v if s > 0 else acc - v
    return acc


def _lhs_ops(top, bot):
    pt = [dict(a=b, b=t, c=t - b) for t, b in zip(top, bot)]
    return (_signed_sum([(pt[k][p], s) for k, p, s in l]) for l, _, _ in _ALG[:15 if len(top) == 3 else 7])


def _rhs_ops(blk):
    n_blk = len(blk)
    wide = [[b.astype(f32) for b in row] for row in blk]
    for _, r, _ in _ALG[:15 if n_blk == 3 else 7]:
        r = [(k, n, s) for k, n, s in r if k < n_blk and n < n_blk]
        yield blk[r[0][0]][r[0][1]] if len(r) == 1 else _signed_sum([(wide[k][n], s) for k, n, s in r]).astype(bf16)


def _signed_add(a, b):
    if a is None:
        return b
    if a[1] == b[1]:
        return a[0] + b[0], a[1]
    return (a[0] - b[0], 1) if a[1] > 0 else (b[0] - a[0], 1)


def _scatter(acc, m, val, tiles):
    for n, p, s in _ALG[m][2]:
        acc[(tiles[n], p)] = _signed_add(acc.get((tiles[n], p)), (val, s))


def _gather(acc, tile):
    out = [_signed_add(acc[(tile, p)], acc[(tile, 'c')]) for p in 'ab']
    assert all(s > 0 for _, s in out)
    return [v for v, _ in out]


class _Tiled:
    def __init__(self, ref):
        self.ref = ref

    def _idx(self, idx):
        r = idx[0]
        r0, r1 = (r.start, r.start + r.size) if isinstance(r, pl.Slice) else r.indices(2 * self.ref.shape[0])[:2]
        return slice(r0 // 2, r1 // 2), idx[1]

    def __getitem__(self, idx):
        return pltpu.bitcast(self.ref[self._idx(idx)], bf16)

    def __setitem__(self, idx, val):
        self.ref[self._idx(idx)] = val if val.dtype == jnp.uint32 else pltpu.bitcast(val, jnp.uint32)


def _gelu(g):
    c0 = float(np.sqrt(2.0 / np.pi))
    t = jnp.tanh(g * (c0 + (c0 * 0.044715) * (g * g)))
    hg = 0.5 * g
    return hg + hg * t


def _gelu_mul(g, u):
    return _gelu(g) * u


def _dot(a, b, dims=_NN):
    return jax.lax.dot_general(a, b, dims, preferred_element_type=f32)


def _t(n):
    return slice(n * 128, (n + 1) * 128)


def _share(tasks, weights):
    cum = np.cumsum((0,) + tuple(weights)) * len(tasks) // sum(weights)
    return [tasks[a:b] for a, b in zip(cum[:-1], cum[1:])]


K1 = [256] * 7 + [128] * 8
O1 = [int(v) for v in np.cumsum([0] + K1)]


def make(NF=384, TM=416, LR=16, SB=3, gord=(0, 1, 3, 4, 5, 6, 2), starts=(3, 5, 7, 10, 12, 19, 23),
         qk_sp=(1, 1, 1, 1, 1), pv_sp=(2, 3, 1), ln_sp=(3, 2), o_sp=(3, 1), cut2=(13, 8), span=0.98, sp2=0.75,
         p1_sp=(2, 2, 1, 1, 2, 1, 2, 3), q0_sp=(3, 1), v0_sp=(2, 1), x0_sp=(0, 1),
         PR=64, WR=32, sps=(0.6, 0.7, 0.9, 0.9), NE=2,
         span0=0.8, span1=0.85, span2=0.97, span3=0.2, dl=(('n', 20), ('h', 20), ('p', 12), ('s', 32))):
    nt = (S - NF) // TM
    assert NF + nt * TM == S
    TX = max(NF, TM)
    HM = TM // 2
    scale = DH ** -0.5
    c_exp = scale * float(np.log2(np.e))
    P = functools.partial

    def kernel(x_hbm, wqkv_hbm, wo_hbm, wg_hbm, wu_hbm, wd_hbm, o_hbm,
               x_s, o_s, wqkv, wo_raw, wo_f, wgu, wt, wd, wp, wop, r_dn, b1n, b1t, b2, b2x,
               xn0, a1, a2a, a2c, a2x, a2xo, a2r, h0, h0o, h_s, ao, l_s, p_s, y_s, xn_s, pr, q_s, k_s, v_s, qkv_0, y_0, p_0,
               sem_i, sem_o):
        wp = [_Tiled(r) for r in wp]
        wop, r_dn, b1n, b1t, b2, b2x, xn0, a1, a2a, a2c, a2x, a2xo, a2r, h0, h0o = map(
            _Tiled, (wop, r_dn, b1n, b1t, b2, b2x, xn0, a1, a2a, a2c, a2x, a2xo, a2r, h0, h0o))
        copies = []

        def fetch(src, dst):
            copies.append(pltpu.make_async_copy(src, dst, sem_i.at[len(copies)]))
            return copies[-1]

        def fetch_rows(src, dst, r, n):
            return fetch(src.at[pl.ds(r, n)], dst.at[pl.ds(r, n)])

        def fetch_gu(g, r=0, n=384):
            return [fetch(src.at[pl.ds(g * 384 + r, n)], wgu[g].at[pl.ds(o + r, n)])
                    for src, o in ((wg_hbm, 0), (wu_hbm, 384))]

        def fetch_qkv(p):
            return fetch(wqkv_hbm.at[:, pl.ds(p * D, D)], wqkv[p].at[pl.ds(0, D)])
        cp_x0 = fetch_rows(x_hbm, x_s, 0, NF)
        cp_g0 = fetch_gu(0, 0, 128)
        cp_gu = [fetch_gu(0, 128, 256), fetch_gu(1), fetch_gu(2)]
        cp_qkv = [fetch_qkv(p) for p in range(3)]
        cp_t = [fetch(wg_hbm.at[pl.ds(FM, FT)], wt.at[pl.ds(0, FT)]),
                fetch(wu_hbm.at[pl.ds(FM, FT)], wt.at[pl.ds(FT, FT)]),
                fetch(wg_hbm.at[pl.ds(FG, 128)], wt.at[pl.ds(128, 128)]),
                fetch(wu_hbm.at[pl.ds(FG, 128)], wt.at[pl.ds(256, 128)])]
        cp_gu.append(fetch_gu(3))
        cp_x1 = fetch_rows(x_hbm, x_s, NF, TM)
        cp_d1 = fetch(wd_hbm.at[pl.ds(768, F - 768)], wd[1].at[pl.ds(0, F - 768)])
        cp_wo = fetch(wo_hbm, wo_raw.at[pl.ds(0, D)])
        cp_d0 = fetch(wd_hbm.at[pl.ds(0, 768)], wd[0].at[pl.ds(0, 768)])
        cp_x2 = fetch_rows(x_hbm, x_s, NF + TM, S - NF - TM)

        def cp_o(r, n, s):
            return pltpu.make_async_copy(o_s.at[pl.ds(r, n)], o_hbm.at[pl.ds(r, n)], sem_o.at[s])

        zero = []
        pending = []
        clock = [0.0]
        lags = {}
        made = set()

        def missing(stage, *spans):
            return any((stage, r) not in made for r0, r1 in spans for r in range(max(r0, 0), r1, 8))

        def fence(val, *refs):
            for ref in refs:
                if val is None:
                    return
                ref = ref.ref if isinstance(ref, _Tiled) else ref
                n = 16 if ref.dtype == bf16 else 8
                v = pltpu.bitcast(val[0:16 if val.dtype == bf16 else 8], ref.dtype)
                rows = pl.ds(pl.multiple_of(ref.shape[-2] - n + zero[0], n), n)
                ref[(0,) * (len(ref.shape) - 2) + (rows, slice(0, 128))] = v

        def done(kind, *refs):
            if not lags.get(kind):
                return None
            val = jnp.zeros((8, 128), f32)
            for ref in refs:
                fence(val, ref)
                ref = ref.ref if isinstance(ref, _Tiled) else ref
                val = ref[(0,) * (len(ref.shape) - 2) + (slice(ref.shape[-2] - 8, None), slice(0, 128))]
            return lags[kind], val

        def phase(dots, *task_lists, span=span):
            total = sum(d[1] for d in dots)
            todo = sorted((clock[0] + s / len(ts) * span * total, n, s)
                          for n, ts in enumerate(task_lists) for s in range(len(ts)))
            out = []
            dots = list(dots)
            while dots:
                for due in [d for d in pending if d[0] <= clock[0]]:
                    fence(due[2], dots[0][2])
                pending[:] = [d for d in pending if d[0] > clock[0]]
                cost, first = 0, len(out)
                while dots and cost < 3:
                    cost += dots[0][1]
                    out.append(dots.pop(0)[0]())
                m = out[first]
                for at, n, s in [t for t in todo if t[0] < clock[0] + cost]:
                    r = min(int(max(at - clock[0], 0) / cost * m.shape[0]) // 16 * 16, m.shape[0] - 16)
                    res = task_lists[n][s](m[r:r + 16, 0:128])
                    if res is not _LATER:
                        todo.remove((at, n, s))
                        if res is not None:
                            pending.append((max(at, clock[0]) + res[0], n, res[1]))
                clock[0] += cost
            for _, n, s in todo:
                res = task_lists[n][s](None)
                assert res is not _LATER
            return out

        def perm_qkv(p, n, r0, tok):
            lane = jax.lax.broadcasted_iota(jnp.int32, (32, 128), 1)
            m_of = 4 * (lane % 32) + lane // 32
            fence(tok, wqkv[p])
            for r in range(r0, r0 + n, 64):
                src = [pltpu.bitcast(wqkv[p][r:r + 64, _t(i)], jnp.uint32) for i in range(NT)]
                for j in range(NT):
                    t = src[0]
                    for i in range(1, NT):
                        t = jnp.where(lane % NT == (j - 128 * i) % NT, src[i], t)
                    wp[p][r:r + 64, _t(j)] = jnp.take_along_axis(
                        t, (NT * m_of + j) % 128, axis=1, mode='promise_in_bounds')

        def tail_t(j, tok):
            wp[3][0:D, _t(j)] = wt[_t(j), :].astype(f32).T.astype(bf16)

        def prep1(g, s, r, tok):
            assert ('w', g) in made
            if g < 3:
                fence(tok, wp[g])

                def get(k, n):
                    return wp[(6 * g + n) // NT][pl.ds(r + k * 128, 16), _t((6 * g + n) % NT)]

                def put(ko, n, v):
                    b1n[ko + r:ko + r + 16, _t(3 * g + n)] = v
            else:
                fence(tok, b1t if ('busy', g) in made else wgu[g - 3])

                def get(k, n):
                    return wgu[g - 3][pl.ds(r + n % 2 * 384 + n // 2 * 128, 16), _t(k)]

                def put(ko, n, v):
                    b1t[pl.ds((g - 3) * 384 + n * 128 + r, 16), ko:ko + 128] = v
            todo = ([((0, 1, 2), (s, 2 + s, 4 + s), 0, s)] if s < 2 else
                    [((3, 4), ns, 128, j) for j, ns in enumerate(((0, 2), (1, 3), (4, 5)))])
            for ks, ns, o, j in todo:
                for m, v in enumerate(_rhs_ops([[get(k, n) for n in ns] for k in ks])):
                    put(O1[m] + o, j, v)

        def widen_wo(_, n, r, tok):
            fence(tok, wo_raw)
            v = wo_raw[r:r + n, :].astype(f32)
            for j in range(NT):
                wo_f[j, r:r + n, :] = v[:, _t(j)]

        def perm_wo(j, tok):
            fence(tok, wo_f)
            for r4 in range(4):
                for i in range(NT):
                    wop[j * 128 + r4 * 32:j * 128 + (r4 + 1) * 32, _t(i)] = (
                        wo_f[i, pl.ds(NT * r4 + j, H, stride=DH), :].astype(bf16))

        def prep2(gg, s, r, tok):
            fence(tok, (b2x, wd[1], wop)[gg])

            def get(k, n):
                src, o = (wd[0], k) if k < 6 else (wd[1], k - 6) if k < 13 else (wop, k - 13)
                return src[pl.ds(r + o * 128, 16), _t(n)]
            todo = ([((3 * s, 3 * s + 1, 3 * s + 2), (0, 1, 2), b2, 2 * gg + s, 0)] if s < 2 else
                    [((2, 5), (3, 4), b2x, gg, 0), ((0, 1), (3, 4), b2, 2 * gg, 15), ((3, 4), (3, 4), b2, 2 * gg + 1, 15)])
            for ks, ns, dst, j, c in todo:
                for m, v in enumerate(_rhs_ops([[get(6 * gg + k, n) for n in ns] for k in ks])):
                    dst[pl.ds(j * 128 + r, 16), _t(c + m)] = v

        def ln(r0):
            x = x_s[pl.ds(r0, LR), :].astype(f32)
            xc = x - jnp.sum(x, axis=-1, keepdims=True) * (1.0 / D)
            var = jnp.sum(xc * xc, axis=-1, keepdims=True) * (1.0 / D)
            return xc * jax.lax.rsqrt(var + 1e-5)

        def normalize(base, r, tok):
            fence(tok, x_s)
            xn_s[r:r + LR, :] = v = ln(pl.multiple_of(base + r, 16))
            made.update(('xn', r0) for r0 in range(r, r + LR, 8))
            return done('n', xn_s)

        def x_ops(ks, r, tok):
            if missing('xn', (r, r + 16), (HM + r, HM + r + 16)):
                return _LATER
            fence(tok, xn_s)
            o = 128 if len(ks) == 2 else 0
            for m, a in enumerate(_lhs_ops(*[[xn_s[r0:r0 + 16, _t(k)] for k in ks] for r0 in (r, HM + r)])):
                a1[r:r + 16, O1[m] + o:O1[m] + o + 128] = a.astype(bf16)
        x_tasks = [P(x_ops, ks, r) for r in range(0, HM, 16) for ks in ((0, 1, 2), (3, 4))]

        def gelu_tail(val):
            lane = jax.lax.broadcasted_iota(jnp.int32, val.shape, 1)
            return jnp.where(lane < FT, _gelu_mul(val, pltpu.roll(val, FT, 1)), 0.0)

        def quarters(n):
            lane = jax.lax.broadcasted_iota(jnp.int32, (n, 128), 1)
            return lane, lane % 64 < 32, lane < 64

        def attn_qk(q_s, k_s, r, c, tok):
            if missing(0, (r, r + 8)) or missing(1, (r - HALO, r + 8)):
                return _LATER
            fence(tok, q_s, k_s)
            made.add((('l', c), r))
            _, even, low = quarters(8)
            q = [q_s[j, r:r + 8, :] for j in range(NT)]

            def part(w):
                return functools.reduce(
                    jnp.add, (q[j] * k_s[j, pl.ds(HALO + r - DIL * w, 8), :] for j in range(NT)))

            def fold(sel, a, b, shift):
                return jnp.where(sel, a, b) + pltpu.roll(jnp.where(sel, b, a), shift, 1)
            u = [fold(even, part(w), part(w + 1), 32) for w in (4 * c, 4 * c + 2)]
            l_s[r:r + 8, _t(c)] = fold(low, u[0], u[1], 64)

        def softmax(p_s, rs, first, tok):
            if any(missing(('l', c), (r, r + 16)) for r in rs for c in range(2)):
                return _LATER
            fence(tok, l_s)
            made.update(('p', r + o) for r in rs for o in (0, 8))
            lg = [[l_s[r:r + 16, _t(c)] for r in rs] for c in range(2)]
            if first:
                row = jax.lax.broadcasted_iota(jnp.int32, (16, 128), 0)
                for c in range(2):
                    lg[c][0] = jnp.where(row >= DIL * (4 * c + quarters(16)[0] // 32), lg[c][0], -1e9 / scale)
            lg = [jnp.concatenate(v, axis=0) for v in lg]

            def all_reduce(op, v):
                v = op(v[0], v[1])
                v = op(v, pltpu.roll(v, 64, 1))
                return op(v, pltpu.roll(v, 32, 1))
            mx = all_reduce(jnp.maximum, lg)
            e = [jnp.exp2((v - mx) * c_exp) for v in lg]
            inv = 1.0 / all_reduce(jnp.add, e)
            for c in range(2):
                for n, r in enumerate(rs):
                    p_s[r:r + 16, _t(c)] = e[c][16 * n:16 * n + 16] * inv[16 * n:16 * n + 16]
            return done('s', p_s)

        def logits(q_s, k_s, p_s, rows, first):
            out = []
            for n, r in enumerate(rows + [None]):
                if r is not None:
                    out += [P(attn_qk, q_s, k_s, r + o, c) for o in (0, 8) for c in range(2)]
                if n > 0 and (n % SB == 0 or r is None):
                    n0 = (n - 1) // SB * SB
                    out.append(P(softmax, p_s, rows[n0:n], first and n0 == 0))
            return out

        def attn_pv(p_s, v_s, r, tok):
            if missing('p', (r, r + 8)) or missing(2, (r - HALO, r + 8)):
                return _LATER
            _, even, low = quarters(8)

            def spread(sel, z, shift):
                y = pltpu.roll(z, shift, 1)
                return jnp.where(sel, z, y), jnp.where(sel, y, z)
            fence(tok, p_s)
            p = [b for c in range(2) for a in spread(low, p_s[r:r + 8, _t(c)], 64) for b in spread(even, a, 32)]
            fence(p[0], v_s)
            for j in range(NT):
                ao[r:r + 8, _t(j)] = functools.reduce(
                    jnp.add, (p[w] * v_s[j, pl.ds(HALO + r - DIL * w, 8), :] for w in range(WIN)))
            made.add(('o', r))
            return done('p', ao)

        def attn_ops(s, r, tok):
            if missing('o', (r, r + 16), (HM + r, HM + r + 16)):
                return _LATER
            fence(tok, ao)
            t, b = [[(ao if j < NT else h_s)[pl.ds(r + o, 16), _t(j)] for j in ((12, 0, 1), (2, 3, 4), (1, 4))[s]]
                    for o in (0, HM)]
            for m, a in enumerate(_lhs_ops(t, b)):
                (a2c if s < 2 else a2xo)[r:r + 16, _t(2 * m + s if s < 2 else m)] = a.astype(bf16)

        def tail_op(r, tok):
            fence(tok, h_s)
            a2r[r:r + 32, :] = gelu_tail(h_s[r:r + 32, _t(13)]).astype(bf16)

        def mm1(g):
            def one(ks, n0, n1, c):
                if g < 3:
                    p = _dot(a1[0:HM, ks], b1n[ks, g * 384 + n0:g * 384 + n1])
                else:
                    p = _dot(a1[0:HM, ks], b1t[(g - 3) * 384 + n0:(g - 3) * 384 + n1, ks], _NT)
                pr[gord.index(g) % 2][0:HM, c * 128:c * 128 + n1 - n0] = p
                return p
            return [(P(one, slice(O1[m], O1[m + 1]), 0, 256, 2 * m) if m < 15 else
                     P(one, slice(O1[m - 15] + 128, O1[m - 15] + 256), 256, 384, 15 + m),
                     K1[m] // 64 if m < 15 else 1, b1n if g < 3 else b1t) for m in range(22)]

        def epi1(g, r, j0, j1, acc, res, tok):
            src = pr[gord.index(g) % 2]
            fence(tok, src)
            for j in range(j0, j1):
                s, m = divmod(j - 7, 15)
                if j < 7:
                    _scatter(acc, j, src[r:r + 8, _t(30 + j)], (4, 5))
                    continue
                _scatter(acc, m, src[r:r + 8, _t(2 * m + s)], (s, 2 + s, 4 + s))
                if m < 14:
                    continue
                if s == 1:
                    made.update(((g, r), (g, HM + r)))
                for c in range(s, 6, 2):
                    n = 6 * g + c
                    for r0, val in zip((r, HM + r), _gather(acc, c)):
                        if n < NT:
                            q_s[n, r0:r0 + 8, :] = val
                        elif n < 15:
                            (k_s, v_s)[n // NT - 1][n % NT, HALO + r0:HALO + r0 + 8, :] = val
                        elif n == 15:
                            h_s[r0:r0 + 8, _t(13)] = val
                        elif s == 0:
                            res[(c, r0)] = _gelu(val)
                        else:
                            val = res[(c - 1, r0)] * val
                            h_s[r0:r0 + 8, _t(12 if g == 2 else n // 2 - 9)] = val

        def h_ops(g, r, tok):
            fence(tok, h_s)
            t, b = [[h_s[pl.ds(r + o, 16), _t(3 * g + k)] for k in range(3)] for o in (0, HM)]
            for m, a in enumerate(_lhs_ops(t, b)):
                a2a[r:r + 16, _t(4 * m + g)] = a.astype(bf16)
            if g % 2 == 1:
                t0, b0 = [h_s[pl.ds(r + o, 16), _t(3 * g - 1)] for o in (0, HM)]
                for m, a in enumerate(_lhs_ops([t0, t[2]], [b0, b[2]])):
                    a2x[r:r + 16, _t(2 * m + g // 2)] = a.astype(bf16)
            return done('h', *[a2a] + [a2x] * (g % 2))

        def epis(g):
            out = []
            for r in range(0, HM + 16, 16):
                if r < HM:
                    for r0, state in ((r, ({}, {})), (r + 8, ({}, {}))):
                        out += [P(epi1, g, r0, a, b, *state) for a, b in ((0, 22), (22, 37))]
                if g >= 3 and r >= 16:
                    out.append(P(h_ops, g - 3, r - 16))
            return out

        def outputs(base):
            return [P(epi2, base, s, r) for r in range(0, HM, 16) for s in range(2)]

        def epi2(base, s, r, tok):
            src, n_prod, tiles = pr[2 + s], (15, 7)[s], ((0, 1, 2), (3, 4))[s]
            fence(tok, src, y_s)
            acc = {}
            for m in range(n_prod):
                _scatter(acc, m, src[r:r + 16, _t(m)], tiles)
            for n in tiles:
                for o, val in zip((r, HM + r), _gather(acc, n)):
                    rows = pl.ds(pl.multiple_of(base + o, 16), 16)
                    o_s[rows, _t(n)] = (val + y_s[o:o + 16, _t(n)]).astype(bf16)

        def tile(i, carry):
            base = pl.multiple_of(NF + i * TM, 32)
            nxt = NF + jnp.minimum(i + 1, nt - 1) * TM
            k_s[:, 0:HALO, :] = k_s[:, TM:TM + HALO, :]
            v_s[:, 0:HALO, :] = v_s[:, TM:TM + HALO, :]
            rows = sorted(range(0, TM, 16), key=lambda r: r % HM or HM // 2)
            qk = _share(logits(q_s, k_s, p_s, rows, False), qk_sp)
            rows = sorted(range(0, HM, 16), key=lambda r: r or HM // 2)
            pv = _share([P(attn_pv, p_s, v_s, o + r) for r in rows for o in (0, 8, HM, HM + 8)], pv_sp)
            cb = _share([P(attn_ops, s, r) for r in rows for s in range(3)], (1, 1))
            lns = _share([P(normalize, nxt, r) for r in range(0, TM, LR)], ln_sp)
            pending.clear()
            made.clear()
            prev = pl.multiple_of(jnp.maximum(base - TM, 0), 32)
            outs = _share(outputs(prev), o_sp)
            phase(mm1(0), lns[0], outs[0])
            phase(mm1(1), epis(0), lns[1], outs[1])
            idle = [lambda tok: None] * 2
            for n in range(2, 7):
                phase(mm1(gord[n]), epis(gord[n - 1]), idle * (3 * (n == 2)) + qk[n - 2])

            def mm2(m, n, acc, dst, lhs, rhs):
                p = _dot(jnp.concatenate([a[0:HM, (w * m + w0) * 128:(w * m + w1) * 128] for a, w, w0, w1 in lhs], axis=1),
                         jnp.concatenate([b[k0:k1, _t(c + m)] for b, k0, k1, c in rhs], axis=0))
                p = p if acc is None else acc[n] + p
                if dst is not None:
                    dst[0:HM, _t(m)] = p
                return p

            def mm2s(ms, *a):
                return [(P(mm2, m, n, *a), sum(w1 - w0 for _, _, w0, w1 in a[2]), b2) for n, m in enumerate(ms)]
            d = mm2s(range(15), None, None, [(a2a, 4, 0, 4)], [(b2, 0, 512, 0)])
            p = phase(d[:cut2[0]], epis(2), idle + pv[0], span=1)
            d = d[cut2[0]:] + mm2s(range(7), None, None, [(a2a, 4, 0, 4)], [(b2, 0, 512, 15)])
            p += phase(d[:cut2[1]], pv[1], cb[0], [P(tail_op, r) for r in range(0, TM, 32)], span=1)

            def tail():
                y_s[0:TM, :] = y = _dot(a2r[:, :], r_dn[:, :]) + x_s[pl.ds(base, TM), :].astype(f32)
                return y
            p += phase(d[cut2[1]:] + mm2s(range(7), None, None, [(a2x, 2, 0, 2)], [(b2x, 0, 256, 0)])
                       + [(tail, 10, b2)],
                       pv[2] + idle * 2, cb[1], span=sp2)
            phase(mm2s(range(15), p, pr[2], [(a2c, 2, 0, 2)], [(b2, 512, 768, 0)]), x_tasks, span=1)
            phase(mm2s(range(7), [p[15 + m] + p[22 + m] for m in range(7)], pr[3],
                       [(a2c, 2, 0, 2), (a2xo, 1, 0, 1)], [(b2, 512, 768, 15), (b2x, 256, 384, 0)]))
            pl.when(i > 0)(lambda: cp_o(prev, TM, i - 1).start())
            return carry

        batches = [copies[a:b] for a, b in zip((0,) + starts, starts)]

        def wait(*cs):
            pending.clear()
            for c in batches.pop(0) if batches else ():
                c.start()
            for c in cs:
                assert not any(c is b for batch in batches for b in batch) and starts[-1] == len(copies)
                c.wait()
        wait()
        for ref in (pr[2], pr[3], y_s):
            ref[...] = jnp.zeros(ref.shape, f32)
        wait(cp_x0)
        bits = jax.lax.population_count(jax.lax.bitcast_convert_type(x_s[0:16, 0:128].astype(f32), jnp.int32))
        zero.append(bits[0, 0] >> 6)
        for r in range(0, NF, LR):
            xn0[r:r + LR, :] = ln(r).astype(bf16)

        def strips(f, a, n):
            return [P(f, a, n, r) for r in range(0, D, n)]

        def prep(f, a):
            return [P(f, a, s, r) for r in range(0, 128, 16) for s in range(3)]

        def dot0(w, dims, finish):
            res = _dot(xn0[:, :], w(), dims)
            finish(res)
            return res

        def gu0(g):
            made.difference_update(('busy', n) for n in range(7))
            made.update((('busy', g + 3), ('w', g + 3)))

            def finish(k, res):
                h0[:, _t(3 * g + k)] = _gelu_mul(res[:, :128], res[:, 128:]).astype(bf16)
            return [(P(dot0, lambda k=k: jnp.concatenate([wgu[g][_t(k), :], wgu[g][_t(3 + k), :]], axis=0), _NT,
                       P(finish, k)), 10, wgu[g]) for k in range(3)]

        def qkv0(p):
            def finish(j, res):
                qkv_0[p][j, HALO * (p > 0):HALO * (p > 0) + NF, :] = res
                if p > 0:
                    qkv_0[p][j, 0:HALO, :] = jnp.broadcast_to(res[0:1], (HALO, 128))
                    (k_s, v_s)[p - 1][j, TM:TM + HALO, :] = res[NF - HALO:]
            return [(P(dot0, lambda j=j: wp[p][0:D, _t(j)], _NN, P(finish, j)), 5, wp[p]) for j in range(NT)]

        def tail0(res):
            h0[:, _t(12)] = _gelu_mul(res[:, _t(1)], res[:, _t(2)]).astype(bf16)
            h0[:, _t(13)] = gelu_tail(res[:, _t(0)]).astype(bf16)

        def down0(acc, a, k0, k1, b):
            return [(lambda j=j: acc(j) + _dot(a[0:NF, k0:k1], b[0:k1 - k0, _t(j)]), (k1 - k0) // 128, b)
                    for j in range(NT)]

        def attn0(r, tok):
            if missing('o', (r, r + 16)):
                return _LATER
            h0o[r:r + 16, :] = ao[r:r + 16, :].astype(bf16)
        pv = _share([P(attn_pv, p_0, qkv_0[2], r) for r in range(0, NF, 8)]
                    + [P(attn0, r) for r in range(0, NF, 16)], v0_sp)
        xs = _share(x_tasks, x0_sp)
        nrm = [P(normalize, NF, r) for r in range(0, TM, LR)]
        p1 = _share(prep(prep1, 3) + prep(prep1, 4) + prep(prep1, 5) + prep(prep1, 0) + prep(prep1, 1)
                    + prep(prep1, 6) + prep(prep1, 2), p1_sp)
        wait(*cp_g0)
        phase(gu0(0)[:1])
        wait(*cp_gu[0])
        phase(gu0(0)[1:], p1.pop(0), span=span0)
        wait(*cp_gu[1])
        phase(gu0(1), p1[0], span=span0)
        wait(*cp_gu[2], cp_qkv[0])
        phase(gu0(2), strips(perm_qkv, 0, PR), p1[1], span=span1)
        wait(*cp_qkv[1:])
        phase(qkv0(0), strips(perm_qkv, 1, PR), p1[2], span=span0)
        made.add(('w', 0))
        phase(qkv0(1), strips(perm_qkv, 2, PR), p1[3], span=sps[0])
        made.add(('w', 1))
        made.update((g, r) for g in range(3) for r in range(0, NF, 8))
        qk = _share(logits(*qkv_0[:2], p_0, list(range(0, NF, 16)), True), q0_sp)
        phase(qkv0(2), p1[4], qk[0], span=sps[1])
        wait(*cp_t, *cp_gu[3], cp_x1)
        made.update(('w', g) for g in range(7))
        phase(gu0(3) + [(P(dot0, lambda: wt[...], _NT, tail0), 15, wgu[3])], nrm, qk[1],
              [P(tail_t, j) for j in range(3)] + p1[5], span=sps[2])
        wait(cp_d1, cp_wo, cp_d0, cp_x2)
        r_dn[0:FT, :] = wd[1][FM - 768:F - 768, :]
        r_dn[FT:, :] = jnp.zeros((128 - FT, D), bf16)
        y = phase([(lambda j=j: x_s[0:NF, _t(j)].astype(f32) + _dot(h0[:, 768:], jnp.concatenate(
            [wd[1][0:FM - 768, _t(j)], r_dn[:, _t(j)]], axis=0)), 8, None) for j in range(NT)],
                  strips(widen_wo, 0, WR) + [P(perm_wo, j) for j in range(NT)], xs[0], p1[6],
                  pv[0], span=sps[3])
        y = phase(down0(y.__getitem__, h0, 0, 768, wd[0]),
                  prep(prep2, 0), prep(prep2, 1) + prep(prep2, 2), xs[1], pv[1], span=span2)
        for j in range(NT):
            y_0[:, _t(j)] = y[j]
        lags.update(dl)
        jax.lax.fori_loop(0, nt, tile, None)

        pending.clear()
        cp_last = [pltpu.make_async_copy(o_s.at[pl.ds(0, NF), _t(j)], o_hbm.at[pl.ds(0, NF), _t(j)], sem_o.at[nt + j])
                   for j in range(NT)]
        dots = down0(lambda j: y_0[:, _t(j)], h0o, 0, D, wop)
        y = phase(dots[:NE], outputs(S - TM), span=span3)
        cp_o(S - TM, TM, nt - 1).start()
        for j in range(NT):
            o_s[0:NF, _t(j)] = (y[j] if j < NE else dots[j][0]()).astype(bf16)
            cp_last[j].start()
        for c in [cp_o(NF + i * TM, TM, i) for i in range(nt)] + cp_last:
            c.wait()

    def fn(A_x, A_wqkv, A_wo, B_x, B_w_gate, B_w_up, B_w_down):
        hbm = pl.BlockSpec(memory_space=pl.ANY)
        V = pltpu.VMEM

        def T(rows, panels):
            return V((rows // 2, panels * 128), jnp.uint32)
        out = pl.pallas_call(
            kernel,
            in_specs=[hbm] * 6,
            out_specs=hbm,
            out_shape=jax.ShapeDtypeStruct((S, D), A_x.dtype),
            scratch_shapes=[
                V((S + 16, D), bf16), V((S + 16, D), bf16), [V((D + 16, D), bf16)] * 3, V((D + 16, D), bf16),
                V((NT, D + 32, 128), f32), [V((768 + 16, D), bf16)] * 4, V((384, D), bf16),
                [V((F - 768 + 16, D), bf16)] * 2, [T(D + 16, NT)] * 4, T(D + 16, NT), T(128, NT),
                T(O1[15] + 16, 9), T(FG + 16, 22), T(768 + 16, 22), T(384 + 16, 7),
                T(NF, NT), T(HM + 16, 22), T(HM + 16, 60), T(HM + 16, 30),
                T(HM + 16, 14), T(HM + 16, 7), T(TM, 1),
                T(NF, 14), T(NF, NT), V((TM + 8, 14 * 128), f32), V((TX + 8, D), f32),
                V((TX + 8, 256), f32), V((TM + 8, 256), f32), V((TM + 8, D), f32), V((TM + 8, D), f32),
                [V((HM + 8, n * 128), f32) for n in (37, 37, 15, 7)],
                V((NT, TM + 8, 128), f32), V((NT, HALO + TM + 8, 128), f32), V((NT, HALO + TM + 8, 128), f32),
                [V((NT, HALO + NF + 8, 128), f32)] * 3, V((NF, D), f32), V((NF + 8, 256), f32),
                pltpu.SemaphoreType.DMA((23,)), pltpu.SemaphoreType.DMA((nt + NT,)),
            ],
            compiler_params=pltpu.CompilerParams(vmem_limit_bytes=110 * 1024 * 1024),
        )(A_x.reshape(S, D), A_wqkv, A_wo, B_w_gate.T, B_w_up.T, B_w_down)
        return out.reshape(A_x.shape)
    return fn


_kernel_fn = make()


@jax.jit
def pallas_parallel_sum__sliding_local_dilated__geglu_ffn__prompt_kernel(
    A_x: jax.Array,
    A_wqkv: jax.Array,
    A_wo: jax.Array,
    B_x: jax.Array,
    B_w_gate: jax.Array,
    B_w_up: jax.Array,
    B_w_down: jax.Array,
):
    return _kernel_fn(A_x, A_wqkv, A_wo, B_x, B_w_gate, B_w_up, B_w_down)
```
